```python
import os as _os
_os.environ.setdefault("JAX_PLATFORMS", "cpu")
import jax
import jax.numpy as jnp

def _softmax(x, axis=-1):
    return jax.nn.softmax(x, axis=axis)
def _gelu(x):
    return jax.nn.gelu(x, approximate=True)
def _silu(x):
    return jax.nn.silu(x)
def _sigmoid(x):
    return jax.nn.sigmoid(x)
def _layernorm(x, axis=-1, eps=1e-5):
    m = jnp.mean(x, axis=axis, keepdims=True)
    v = jnp.var(x, axis=axis, keepdims=True)
    return (x - m) / jnp.sqrt(v + eps)
def _scatter_add(tgt, idx, src, axis=0):
    return tgt.at[idx].add(src)
def _segment_sum(src, seg, n):
    return jax.ops.segment_sum(src, seg, n)
class _Rng:
    def __init__(self, key):
        self._k = key
    def _next(self):
        self._k, sub = jax.random.split(self._k)
        return sub
    def normal(self, shape):
        return jax.random.normal(self._next(), shape, dtype=jnp.bfloat16)
    def randint(self, lo, hi, shape):
        return jax.random.randint(self._next(), shape, lo, hi, dtype=jnp.int32)
    def uniform(self, shape, lo=0.0, hi=1.0):
        return jax.random.uniform(self._next(), shape, jnp.bfloat16, lo, hi)
    def permutation(self, n):
        return jax.random.permutation(self._next(), n)


kernel_name = 'parallel_sum__ssm_conv_h3__dense_activation_silu__prompt'

def setup_inputs():
    _rng = _Rng(jax.random.key(int.from_bytes(__import__("os").urandom(4), "little")))
    _w = (lambda a: (lambda t: t.astype(jnp.bfloat16) if jnp.issubdtype(t.dtype, jnp.floating) else t)(jnp.asarray(a)))
    def _A_setup():
        B, S, D = 1, 2048, 448
        ks = 4
        return {
            "q": _w((lambda *s: _rng.normal(s) * 0.05)(B, S, D)),
            "k": _w((lambda *s: _rng.normal(s) * 0.2)(B, S, D)),
            "v": _w((lambda *s: _rng.normal(s) * 0.2)(B, S, D)),
            "shift_k": _w((lambda *s: _rng.normal(s) * 0.2)(D, ks) * 0.5),
            "ssm_k": _w((lambda *s: _rng.normal(s) * 0.2)(D, S) * (1.0 / S ** 0.5)),
            "ssm_D": _w((lambda *s: _rng.normal(s) * 0.2)(D)),
        }
    _A_in = _A_setup()

    def _B_setup():
        B, S, D, F = 1, 2048, 448, 1792
        return {
            "x": _w((lambda *s: _rng.normal(s) * 0.05)(B, S, D)),
            "w1": _w((lambda *s: _rng.normal(s) * 0.05)(D, F) * (D ** -0.5)),
            "w2": _w((lambda *s: _rng.normal(s) * 0.05)(F, D) * (F ** -0.5)),
        }
    _B_in = _B_setup()

    return {
        "A_q": _A_in["q"],
        "A_k": _A_in["k"],
        "A_v": _A_in["v"],
        "A_shift_k": _A_in["shift_k"],
        "A_ssm_k": _A_in["ssm_k"],
        "A_ssm_D": _A_in["ssm_D"],
        "B_x": _B_in["x"],
        "B_w1": _B_in["w1"],
        "B_w2": _B_in["w2"],
    }

def reference(A_q, A_k, A_v, A_shift_k, A_ssm_k, A_ssm_D, B_x, B_w1, B_w2):
    def _A_ref(q, k, v, shift_k, ssm_k, ssm_D):
        B, S, D = q.shape
        ks = shift_k.shape[-1]
        k_pad = jnp.pad(k, ((0, 0), (ks - 1, 0), (0, 0)))
        k_shift = jnp.zeros_like(k)
        for t in range(ks):
            k_shift = k_shift + k_pad[:, t:t + S, :] * shift_k[:, ks - 1 - t][None, None, :]
        kv = k_shift * v
        L = 2 * S
        kv_pad = jnp.pad(kv, ((0, 0), (0, S), (0, 0)))
        kf_pad = jnp.pad(ssm_k, ((0, 0), (0, S)))
        kv_f = (lambda x, axes=(-2,-1): jnp.fft.rfft2(x.astype(jnp.float32), axes=axes))(kv_pad[:, None, :, :], axes=(1, 2))
        kf_f = (lambda x, axes=(-2,-1): jnp.fft.rfft2(x.astype(jnp.float32), axes=axes))(kf_pad[:, None, :], axes=(1, 2))
        kf_f = (lambda x, *d: x.transpose(*d))(kf_f, 1, 2, 0)
        y_f = kv_f * kf_f[None, :, :, :]
        y = (lambda x, s, axes=(-2,-1): jnp.fft.irfft2(x, s=s, axes=axes).astype(jnp.bfloat16))(y_f, (1, L), axes=(1, 2))[:, 0, :S, :]
        y = y + kv * ssm_D[None, None, :]
        return q * y

    def _B_ref(x, w1, w2):
        h = jnp.einsum("bsd,df->bsf", x, w1)
        h = _silu(h)
        out = jnp.einsum("bsf,fd->bsd", h, w2)
        return out

    x = A_q
    xn = _layernorm(x, axis=-1)
    return x + _A_ref(xn, A_k, A_v, A_shift_k, A_ssm_k, A_ssm_D) + _B_ref(xn, B_w1, B_w2)
```

```python
import numpy as np
import jax
import jax.numpy as jnp
import jax.experimental.pallas as pl
import jax.experimental.pallas.tpu as pltpu

S, D, FF = 2048, 448, 1792
N = 4096
NF1 = 33
IM = 40
R1 = 80
BF = jnp.bfloat16
F32 = jnp.float32


def _hilo(a):
    a = np.asarray(a, np.float64)
    h = a.astype(jnp.bfloat16)
    l = (a - h.astype(np.float64)).astype(jnp.bfloat16)
    return h, l


def _consts():
    t1 = np.arange(32)
    f1 = np.arange(NF1)
    ang = 2 * np.pi * np.outer(f1, t1) / 64.0
    m1 = np.zeros((R1, 32))
    m1[:NF1] = np.cos(ang)
    m1[IM:IM + NF1] = -np.sin(ang)
    m1h, m1l = _hilo(m1)
    m1c = np.concatenate([m1h, m1l], axis=1)
    t2 = np.arange(64)
    f2 = np.arange(64)
    gf = np.zeros((NF1, 128, 128))
    gi = np.zeros((NF1, 128, 128))
    for a in range(NF1):
        an = 2 * np.pi * (np.outer(a + 64 * f2, t2) % N) / N
        c, s = np.cos(an), -np.sin(an)
        gf[a] = np.block([[c, -s], [s, c]])
        c, s = np.cos(an).T, np.sin(an).T
        gi[a] = np.block([[c, -s], [s, c]])
    def cat3(g):
        h, l = _hilo(g)
        return h
    w = np.full(NF1, 2.0); w[0] = 1.0; w[32] = 1.0
    m2 = np.zeros((32, 2 * IM))
    m2[:, :NF1] = (np.cos(ang) * w[:, None]).T / N
    m2[:, IM:IM + NF1] = (-np.sin(ang) * w[:, None]).T / N
    return m1c, cat3(gf), cat3(gi), cat3(m2)


def _split3(a):
    h = a.astype(BF)
    l = (a - h.astype(F32)).astype(BF)
    return h


def _dot(a, b):
    return jnp.dot(a, b, preferred_element_type=F32)


def _body(q_ref, k_ref, v_ref, sk_ref, kt_ref, sd_ref, w1_ref, w2_ref,
          m1_ref, gf_ref, gi_ref, m2_ref, o_ref,
          kvf_s, kv_s, kk_s, a1_s, a2_s, b_s, y_s):
    TB = 256
    rows = jax.lax.broadcasted_iota(jnp.int32, (TB + 8, D), 0)
    for i in range(S // TB):
        lo = max(i * TB - 8, 0)
        kx = k_ref[pl.ds(lo, TB + 8), :].astype(F32) if i > 0 else None
        if i == 0:
            kx = jnp.concatenate([jnp.zeros((8, D), F32), k_ref[pl.ds(0, TB), :].astype(F32)], axis=0)
        acc = kx[8:, :] * sk_ref[0:1, :]
        for j in range(1, 4):
            acc = acc + pltpu.roll(kx, j, 0)[8:, :] * sk_ref[j:j + 1, :]
        kv = acc.astype(BF).astype(F32) * v_ref[pl.ds(i * TB, TB), :].astype(F32)
        kvf_s[pl.ds(i * TB, TB), :] = kv.astype(BF).astype(F32)
        z = jnp.zeros((TB, 64), F32)
        for val, dst in ((kv.astype(BF).astype(F32), kv_s),
                         (kt_ref[pl.ds(i * TB, TB), :].astype(F32), kk_s)):
            val = jnp.concatenate([val, z], axis=1)
            for c in range(4):
                dst[c, pl.ds(i * TB, TB), :] = val[:, c * 128:(c + 1) * 128]

    m1 = m1_ref[...]

    def s1(t2, c):
        for src, dst in ((kv_s, a1_s), (kk_s, a2_s)):
            for cc in range(4):
                x = src[cc, pl.ds(t2, 32, stride=64), :].astype(BF)
                dst[cc, pl.ds(pl.multiple_of(t2 * R1, 8), R1), :] = _dot(m1, jnp.concatenate([x, x], axis=0))
        return c
    jax.lax.fori_loop(0, 64, s1, 0, unroll=8)

    b_s[:, pl.ds(NF1 * 128, (IM - NF1) * 128), :] = jnp.zeros((4, (IM - NF1) * 128, 128), F32)

    def s2(f1, c):
        g = gf_ref[f1]
        gv = gi_ref[f1]
        for cc in range(4):
            res = []
            for src in (a1_s, a2_s):
                a = jnp.concatenate([src[cc, pl.ds(f1, 64, stride=R1), :],
                                     src[cc, pl.ds(f1 + IM, 64, stride=R1), :]], axis=0)
                res.append(_dot(g, _split3(a)))
            x, k = res
            xr, xi, kr, ki = x[:64], x[64:], k[:64], k[64:]
            y = jnp.concatenate([xr * kr - xi * ki, xr * ki + xi * kr], axis=0)
            b_s[cc, pl.ds(pl.multiple_of(f1 * 128, 128), 128), :] = _dot(gv, _split3(y))
        return c
    jax.lax.fori_loop(0, NF1, s2, 0, unroll=11)

    m2 = m2_ref[...]

    def s3(t2, c):
        for cc in range(4):
            b = jnp.concatenate([b_s[cc, pl.ds(t2, IM, stride=128), :],
                                 b_s[cc, pl.ds(t2 + 64, IM, stride=128), :]], axis=0)
            y_s[cc, pl.ds(t2, 32, stride=64), :] = _dot(m2, _split3(b))
        return c
    jax.lax.fori_loop(0, 64, s3, 0, unroll=8)

    def ffn(i, c):
        r = pl.ds(pl.multiple_of(i * TB, TB), TB)
        x = q_ref[r, :].astype(F32)
        m = jnp.mean(x, axis=-1, keepdims=True)
        xc = x - m
        var = jnp.mean(xc * xc, axis=-1, keepdims=True)
        xn = (xc * jax.lax.rsqrt(var + 1e-5)).astype(BF)
        h = _dot(xn, w1_ref[...]).astype(BF).astype(F32)
        h = (h * jax.nn.sigmoid(h)).astype(BF)
        f = _dot(h, w2_ref[...])
        yc = jnp.concatenate([y_s[0, r, :], y_s[1, r, :], y_s[2, r, :], y_s[3, r, :][:, :64]], axis=1)
        y = yc.astype(BF).astype(F32) + kvf_s[r, :] * sd_ref[...]
        o_ref[r, :] = (x + xn.astype(F32) * y + f).astype(BF)
        return c
    jax.lax.fori_loop(0, S // TB, ffn, 0)


@jax.jit
def pallas_parallel_sum__ssm_conv_h3__dense_activation_silu__prompt_kernel(
    A_q, A_k, A_v, A_shift_k, A_ssm_k, A_ssm_D, B_x, B_w1, B_w2,
):
    m1c, gf, gi, m2 = (jnp.asarray(c) for c in _consts())
    args = (A_q[0], A_k[0], A_v[0], A_shift_k.T.astype(F32), A_ssm_k.T,
            A_ssm_D.reshape(1, D).astype(F32), B_w1, B_w2, m1c, gf, gi, m2)
    out = pl.pallas_call(
        _body,
        out_shape=jax.ShapeDtypeStruct((S, D), BF),
        scratch_shapes=[
            pltpu.VMEM((S, D), F32),
            pltpu.VMEM((4, S, 128), F32), pltpu.VMEM((4, S, 128), F32),
            pltpu.VMEM((4, 64 * R1, 128), F32), pltpu.VMEM((4, 64 * R1, 128), F32),
            pltpu.VMEM((4, IM * 128, 128), F32), pltpu.VMEM((4, S, 128), F32),
        ],
        compiler_params=pltpu.CompilerParams(vmem_limit_bytes=100 * 1024 * 1024),
    )(*args)
    return out[None]
```
